```python
import jax
import jax.numpy as jnp

def _softmax(x, axis=-1):
    return jax.nn.softmax(x, axis=axis)
def _gelu(x):
    return jax.nn.gelu(x, approximate=True)
def _silu(x):
    return jax.nn.silu(x)
def _sigmoid(x):
    return jax.nn.sigmoid(x)
def _layernorm(x, axis=-1, eps=1e-5):
    m = jnp.mean(x, axis=axis, keepdims=True)
    v = jnp.var(x, axis=axis, keepdims=True)
    return (x - m) / jnp.sqrt(v + eps)
def _scatter_add(tgt, idx, src, axis=0):
    return tgt.at[idx].add(src)
def _segment_sum(src, seg, n):
    return jax.ops.segment_sum(src, seg, n)
class _Rng:
    def __init__(self, key):
        self._k = key
    def _next(self):
        self._k, sub = jax.random.split(self._k)
        return sub
    def normal(self, shape):
        return jax.random.normal(self._next(), shape, dtype=jnp.bfloat16)
    def randint(self, lo, hi, shape):
        return jax.random.randint(self._next(), shape, lo, hi, dtype=jnp.int32)
    def uniform(self, shape, lo=0.0, hi=1.0):
        return jax.random.uniform(self._next(), shape, jnp.bfloat16, lo, hi)
    def permutation(self, n):
        return jax.random.permutation(self._next(), n)


kernel_name = 'recurrent_scan__sliding_block_cached__glu_gated_glu__decode'

def setup_inputs():
    _rng = _Rng(jax.random.key(int.from_bytes(__import__("os").urandom(4), "little")))
    _w = (lambda a: (lambda t: t.astype(jnp.bfloat16) if jnp.issubdtype(t.dtype, jnp.floating) else t)(jnp.asarray(a)))
    def _A_setup():
        B, Sq, D = 1, 1, 576
        Hq, Hkv, Sk, Dh = 32, 16, 65536, 128
        assert Hq % Hkv == 0, (Hq, Hkv)
        return {
            "x": _w((lambda *s: _rng.normal(s) * 0.05)(B, Sq, D)),
            "k_cache": _w((lambda *s: _rng.normal(s) * 0.05)(B, Hkv, Sk, Dh)),
            "v_cache": _w((lambda *s: _rng.normal(s) * 0.05)(B, Hkv, Sk, Dh)),
            "wq": _w((lambda *s: _rng.normal(s) * 0.05)(D, Hq * Dh) * (D ** -0.5)),
            "wo": _w((lambda *s: _rng.normal(s) * 0.05)(Hq * Dh, D) * ((Hq * Dh) ** -0.5)),
        }
    _A_in = _A_setup()

    def _B_setup():
        B, S, D, F = 1, 1, 576, 4608
        return {
            "x": _w((lambda *s: _rng.normal(s) * 0.05)(B, S, D)),
            "w_gate": _w((lambda *s: _rng.normal(s) * 0.05)(D, F)),
            "w_up": _w((lambda *s: _rng.normal(s) * 0.05)(D, F)),
            "w_down": _w((lambda *s: _rng.normal(s) * 0.05)(F, D)),
        }
    _B_in = _B_setup()

    return {
        "A_x": _A_in["x"],
        "A_k_cache": _A_in["k_cache"],
        "A_v_cache": _A_in["v_cache"],
        "A_wq": _A_in["wq"],
        "A_wo": _A_in["wo"],
        "B_x": _B_in["x"],
        "B_w_gate": _B_in["w_gate"],
        "B_w_up": _B_in["w_up"],
        "B_w_down": _B_in["w_down"],
    }

def reference(A_x, A_k_cache, A_v_cache, A_wq, A_wo, B_x, B_w_gate, B_w_up, B_w_down):
    def _A_ref(x, k_cache, v_cache, wq, wo):
        B, Sq, D = x.shape
        Hq, Dh = 32, 128
        Hkv, Sk = k_cache.shape[1], k_cache.shape[2]
        W = min(4096, max(256, Sk // 4))
        rep = Hq // Hkv
        q = (lambda x, *d: x.transpose(*d))((x @ wq).reshape(B, Sq, Hq, Dh), 0, 2, 1, 3)
        k = jnp.repeat(k_cache[:, :, Sk - W:, :], rep, axis=1)
        v = jnp.repeat(v_cache[:, :, Sk - W:, :], rep, axis=1)
        scores = jnp.einsum("bhqd,bhkd->bhqk", q, k) * (Dh ** -0.5)
        p = _softmax(scores, axis=-1)
        o = jnp.einsum("bhqk,bhkd->bhqd", p, v)
        return (lambda x, *d: x.transpose(*d))(o, 0, 2, 1, 3).reshape(B, Sq, Hq * Dh) @ wo

    def _B_ref(x, w_gate, w_up, w_down):
        g = jnp.einsum("bsd,df->bsf", x, w_gate)
        u = jnp.einsum("bsd,df->bsf", x, w_up)
        h = _sigmoid(g) * u
        return jnp.einsum("bsf,fd->bsd", h, w_down)

    x = A_x
    xn = _layernorm(x, axis=-1)
    s = _A_ref(xn, A_k_cache, A_v_cache, A_wq, A_wo)
    g = _silu(_B_ref(xn, B_w_gate, B_w_up, B_w_down))
    return x + s * g
```

```python
import jax
import jax.numpy as jnp
from jax import lax
import jax.experimental.pallas as pl
import jax.experimental.pallas.tpu as pltpu

_HQ, _DH = 32, 128
_EPS = 1e-5
_NT = (((1,), (1,)), ((), ()))
_NSEM = 3


def _kernel(x_hbm, k_hbm, v_hbm, wq_hbm, wo_hbm, wg_hbm, wu_hbm, wd_hbm, o_ref,
            x_v, k_v, v_v, wq_v, wo_v, wg_v, wu_v, wd_v, q_s, sems):
    hkv, win, _ = k_v.shape
    start = k_hbm.shape[2] - win
    d = x_v.shape[1]
    last = hkv - 1
    vsplit = (win // 2, win // 4, win // 4)
    voff = (0, win // 2, 3 * win // 4)
    base = 6

    def copy(src, dst, i):
        return pltpu.make_async_copy(src, dst, sems.at[i % _NSEM])

    cx = copy(x_hbm.at[0], x_v, 0)
    cwq = copy(wq_hbm, wq_v, 1)
    cwg = copy(wg_hbm, wg_v, 2)
    cwu = copy(wu_hbm, wu_v, 3)
    cwd = copy(wd_hbm, wd_v, 4)
    cwo = copy(wo_hbm, wo_v, 5)
    ck = lambda h: copy(k_hbm.at[0, h, pl.ds(start, win), :], k_v.at[h], base + 2 * h)
    cv = lambda h: copy(v_hbm.at[0, h, pl.ds(start, win), :], v_v.at[h], base + 2 * h + 1)
    cvl = [
        copy(v_hbm.at[0, last, pl.ds(start + voff[i], vsplit[i]), :],
             v_v.at[last, pl.ds(voff[i], vsplit[i])], base + 2 * last + 1 + i)
        for i in range(3)
    ]

    cx.start()
    cwq.start()
    cx.wait()
    cwg.start()
    x = x_v[...].astype(jnp.float32)
    xc = x - jnp.mean(x, axis=-1, keepdims=True)
    var = jnp.mean(xc * xc, axis=-1, keepdims=True)
    xn = jnp.broadcast_to(xc / jnp.sqrt(var + _EPS), (8, d)).astype(jnp.bfloat16)

    cwq.wait()
    cwu.start()
    q = jnp.dot(xn, wq_v[...], preferred_element_type=jnp.float32)
    q = q.astype(jnp.bfloat16).astype(jnp.float32)
    even = (lax.broadcasted_iota(jnp.int32, (8, _DH), 0) & 1) == 0
    for g in range(hkv):
        q_s[g] = jnp.where(even, q[:, 2 * g * _DH:(2 * g + 1) * _DH],
                           q[:, (2 * g + 1) * _DH:(2 * g + 2) * _DH])

    cwg.wait()
    cwd.start()
    gt = jnp.dot(xn, wg_v[...], preferred_element_type=jnp.float32)
    cwu.wait()
    cwo.start()
    up = jnp.dot(xn, wu_v[...], preferred_element_type=jnp.float32)
    h = (jax.nn.sigmoid(gt) * up).astype(jnp.bfloat16)
    cwd.wait()
    ck(0).start()
    cv(0).start()
    y = lax.dot_general(h, wd_v[...], _NT, preferred_element_type=jnp.float32)
    gate = y * jax.nn.sigmoid(y)
    cwo.wait()
    ck(1).start()

    def probs(g):
        s = lax.dot_general(q_s[g].astype(jnp.bfloat16), k_v[g], _NT,
                            preferred_element_type=jnp.float32) * (_DH ** -0.5)
        p = jnp.exp(s - jnp.max(s, axis=-1, keepdims=True))
        return p.astype(jnp.bfloat16), 1.0 / jnp.sum(p, axis=-1, keepdims=True)

    def project(o, wo_blk):
        o2 = jnp.concatenate([o, pltpu.roll(o, 7, 0)], axis=1).astype(jnp.bfloat16)
        return lax.dot_general(o2, wo_blk, _NT, preferred_element_type=jnp.float32)

    def head(g, acc):
        ck(g).wait()

        @pl.when(g + 1 < last)
        def _():
            cv(g + 1).start()

        @pl.when(g + 1 == last)
        def _():
            cvl[0].start()

        p, inv_l = probs(g)
        cv(g).wait()

        @pl.when(g + 2 < hkv)
        def _():
            ck(g + 2).start()

        @pl.when(g + 2 == hkv)
        def _():
            cvl[1].start()

        o = jnp.dot(p, v_v[g], preferred_element_type=jnp.float32) * inv_l
        col = pl.multiple_of(g * 2 * _DH, 2 * _DH)
        return acc + project(o, wo_v[:, pl.ds(col, 2 * _DH)])

    acc = lax.fori_loop(0, last, head, jnp.zeros((8, d), jnp.float32))

    ck(last).wait()
    cvl[2].start()
    p, inv_l = probs(last)
    o = jnp.zeros((8, _DH), jnp.float32)
    for i in range(3):
        cvl[i].wait()
        rows = slice(voff[i], voff[i] + vsplit[i])
        o = o + jnp.dot(p[:, rows], v_v[last, rows, :], preferred_element_type=jnp.float32)
    s_out = acc + project(o * inv_l, wo_v[:, last * 2 * _DH:])
    o_ref[0] = (x + s_out[0:1] * gate[0:1]).astype(o_ref.dtype)


@jax.jit
def pallas_recurrent_scan__sliding_block_cached__glu_gated_glu__decode_kernel(
    A_x: jax.Array,
    A_k_cache: jax.Array,
    A_v_cache: jax.Array,
    A_wq: jax.Array,
    A_wo: jax.Array,
    B_x: jax.Array,
    B_w_gate: jax.Array,
    B_w_up: jax.Array,
    B_w_down: jax.Array,
):
    del B_x
    d = A_x.shape[-1]
    hkv, sk = A_k_cache.shape[1], A_k_cache.shape[2]
    f = B_w_gate.shape[1]
    win = min(4096, max(256, sk // 4))
    assert A_x.shape == (1, 1, d) and _HQ == 2 * hkv
    hbm = pl.BlockSpec(memory_space=pltpu.HBM)
    return pl.pallas_call(
        _kernel,
        out_shape=jax.ShapeDtypeStruct(A_x.shape, A_x.dtype),
        in_specs=[hbm] * 8,
        out_specs=pl.BlockSpec(memory_space=pltpu.VMEM),
        scratch_shapes=[
            pltpu.VMEM((1, d), A_x.dtype),
            pltpu.VMEM((hkv, win, _DH), A_k_cache.dtype),
            pltpu.VMEM((hkv, win, _DH), A_v_cache.dtype),
            pltpu.VMEM((d, _HQ * _DH), A_wq.dtype),
            pltpu.VMEM((d, _HQ * _DH), A_wo.dtype),
            pltpu.VMEM((d, f), B_w_gate.dtype),
            pltpu.VMEM((d, f), B_w_up.dtype),
            pltpu.VMEM((d, f), B_w_down.dtype),
            pltpu.VMEM((hkv, 8, _DH), jnp.float32),
            pltpu.SemaphoreType.DMA((_NSEM,)),
        ],
        compiler_params=pltpu.CompilerParams(vmem_limit_bytes=100 * 1024 * 1024),
    )(A_x, A_k_cache, A_v_cache, A_wq, A_wo.T, B_w_gate, B_w_up, B_w_down.T)
```
